```python
import jax
import jax.numpy as jnp

def _softmax(x, axis=-1):
    return jax.nn.softmax(x, axis=axis)
def _gelu(x):
    return jax.nn.gelu(x, approximate=True)
def _silu(x):
    return jax.nn.silu(x)
def _sigmoid(x):
    return jax.nn.sigmoid(x)
def _layernorm(x, axis=-1, eps=1e-5):
    m = jnp.mean(x, axis=axis, keepdims=True)
    v = jnp.var(x, axis=axis, keepdims=True)
    return (x - m) / jnp.sqrt(v + eps)
def _scatter_add(tgt, idx, src, axis=0):
    return tgt.at[idx].add(src)
def _segment_sum(src, seg, n):
    return jax.ops.segment_sum(src, seg, n)
class _Rng:
    def __init__(self, key):
        self._k = key
    def _next(self):
        self._k, sub = jax.random.split(self._k)
        return sub
    def normal(self, shape):
        return jax.random.normal(self._next(), shape, dtype=jnp.bfloat16)
    def randint(self, lo, hi, shape):
        return jax.random.randint(self._next(), shape, lo, hi, dtype=jnp.int32)
    def uniform(self, shape, lo=0.0, hi=1.0):
        return jax.random.uniform(self._next(), shape, jnp.bfloat16, lo, hi)
    def permutation(self, n):
        return jax.random.permutation(self._next(), n)


kernel_name = 'sequential_preLN__sliding_block_cached__mixer_s_mlp__decode'

def setup_inputs():
    _rng = _Rng(jax.random.key(int.from_bytes(__import__("os").urandom(4), "little")))
    _w = (lambda a: (lambda t: t.astype(jnp.bfloat16) if jnp.issubdtype(t.dtype, jnp.floating) else t)(jnp.asarray(a)))
    def _A_setup():
        B, Sq, D = 1, 1, 640
        Hq, Hkv, Sk, Dh = 32, 32, 32768, 192
        assert Hq % Hkv == 0, (Hq, Hkv)
        return {
            "x": _w((lambda *s: _rng.normal(s) * 0.05)(B, Sq, D)),
            "k_cache": _w((lambda *s: _rng.normal(s) * 0.05)(B, Hkv, Sk, Dh)),
            "v_cache": _w((lambda *s: _rng.normal(s) * 0.05)(B, Hkv, Sk, Dh)),
            "wq": _w((lambda *s: _rng.normal(s) * 0.05)(D, Hq * Dh) * (D ** -0.5)),
            "wo": _w((lambda *s: _rng.normal(s) * 0.05)(Hq * Dh, D) * ((Hq * Dh) ** -0.5)),
        }
    _A_in = _A_setup()

    def _B_setup():
        B, S, D, F = 1, 1, 640, 1536
        return {
            "x":  _w((lambda *s: _rng.normal(s) * 0.05)(B, S, D)),
            "w1": _w((lambda *s: _rng.normal(s) * 0.05)(D, D) * (D ** -0.5)),
            "w2": _w((lambda *s: _rng.normal(s) * 0.05)(D, D) * (D ** -0.5)),
            "w3": _w((lambda *s: _rng.normal(s) * 0.05)(D, F) * (D ** -0.5)),
            "w4": _w((lambda *s: _rng.normal(s) * 0.05)(F, D) * (F ** -0.5)),
        }
    _B_in = _B_setup()

    return {
        "A_x": _A_in["x"],
        "A_k_cache": _A_in["k_cache"],
        "A_v_cache": _A_in["v_cache"],
        "A_wq": _A_in["wq"],
        "A_wo": _A_in["wo"],
        "B_x": _B_in["x"],
        "B_w1": _B_in["w1"],
        "B_w2": _B_in["w2"],
        "B_w3": _B_in["w3"],
        "B_w4": _B_in["w4"],
    }

def reference(A_x, A_k_cache, A_v_cache, A_wq, A_wo, B_x, B_w1, B_w2, B_w3, B_w4):
    def _A_ref(x, k_cache, v_cache, wq, wo):
        B, Sq, D = x.shape
        Hq, Dh = 32, 192
        Hkv, Sk = k_cache.shape[1], k_cache.shape[2]
        W = min(4096, max(256, Sk // 4))
        rep = Hq // Hkv
        q = (lambda x, *d: x.transpose(*d))((x @ wq).reshape(B, Sq, Hq, Dh), 0, 2, 1, 3)
        k = jnp.repeat(k_cache[:, :, Sk - W:, :], rep, axis=1)
        v = jnp.repeat(v_cache[:, :, Sk - W:, :], rep, axis=1)
        scores = jnp.einsum("bhqd,bhkd->bhqk", q, k) * (Dh ** -0.5)
        p = _softmax(scores, axis=-1)
        o = jnp.einsum("bhqk,bhkd->bhqd", p, v)
        return (lambda x, *d: x.transpose(*d))(o, 0, 2, 1, 3).reshape(B, Sq, Hq * Dh) @ wo

    def _B_ref(x, w1, w2, w3, w4):
        B, S, D = x.shape
        h = _gelu(_layernorm(x, axis=-1) @ w1)
        c = D // 4
        g0 = jnp.pad(h[:, :, 0*c:1*c], ((0, 0), (1, 0), (0, 0)))[:, :S, :]
        g1 = jnp.pad(h[:, :, 1*c:2*c], ((0, 0), (0, 1), (0, 0)))[:, 1:, :]
        g2 = jnp.pad(h[:, :, 2*c:3*c], ((0, 0), (2, 0), (0, 0)))[:, :S, :]
        g3 = jnp.pad(h[:, :, 3*c:   ], ((0, 0), (0, 2), (0, 0)))[:, 2:, :]
        hs = jnp.concatenate([g0, g1, g2, g3], axis=-1) @ w2
        x1 = x + hs
        h2 = _gelu(_layernorm(x1, axis=-1) @ w3) @ w4
        return x1 + h2

    x = A_x
    h = x + _A_ref(_layernorm(x, axis=-1), A_k_cache, A_v_cache, A_wq, A_wo)
    h2 = h + _B_ref(_layernorm(h, axis=-1), B_w1, B_w2, B_w3, B_w4)
    return h2
```

```python
import functools

import jax
import jax.numpy as jnp
import numpy as np
import jax.experimental.pallas as pl
import jax.experimental.pallas.tpu as pltpu

_H, _DH, _D, _F = 32, 192, 640, 1536
_M = 8
_EPS = 1e-5
_SLOTS = 4
_W4_CHUNKS = 2


def _ln(v):
    m = jnp.mean(v, axis=-1, keepdims=True)
    d = v - m
    var = jnp.mean(d * d, axis=-1, keepdims=True)
    return d * jax.lax.rsqrt(var + _EPS)


def _gelu(v):
    c = float(np.sqrt(2.0 / np.pi))
    return 0.5 * v * (1.0 + jnp.tanh(c * (v + 0.044715 * (v * v * v))))


def _kernel(x_hbm, kt_hbm, vt_hbm, wq_hbm, wo_hbm, w3_hbm, w4_hbm, out_ref,
            x_buf, wq_buf, k_buf, v_buf, wo_buf, w3_buf, w4_buf, q_scr, sems, *, sk, w):
    S = _SLOTS
    scale = _DH ** -0.5

    def k_copy(h, slot):
        return pltpu.make_async_copy(kt_hbm.at[h, :, pl.ds(sk - w, w)], k_buf.at[slot], sems.at[slot])

    def v_copy(h, slot):
        return pltpu.make_async_copy(vt_hbm.at[h, :, pl.ds(sk - w, w)], v_buf.at[slot], sems.at[S + slot])

    def wo_copy(h, slot):
        start = h * _DH if isinstance(h, int) else pl.multiple_of(h * _DH, _DH)
        return pltpu.make_async_copy(wo_hbm.at[pl.ds(start, _DH), :], wo_buf.at[slot], sems.at[2 * S + slot])

    x_copy = pltpu.make_async_copy(x_hbm, x_buf, sems.at[3 * S])
    wq_copy = pltpu.make_async_copy(wq_hbm, wq_buf, sems.at[3 * S + 1])
    w3_copy = pltpu.make_async_copy(w3_hbm, w3_buf, sems.at[3 * S + 2])
    rows4 = _F // _W4_CHUNKS

    def w4_copy(c):
        rows = pl.ds(c * rows4, rows4)
        return pltpu.make_async_copy(w4_hbm.at[rows, :], w4_buf.at[rows, :], sems.at[3 * S + 3 + c])

    x_copy.start()
    wq_copy.start()
    for h in range(S):
        k_copy(h, h).start()
        v_copy(h, h).start()
        wo_copy(h, h).start()

    x_copy.wait()
    x8 = jnp.broadcast_to(x_buf[0].astype(jnp.float32), (_M, _D))
    xn = _ln(x8).astype(jnp.bfloat16)
    wq_copy.wait()
    q_all = jnp.dot(xn, wq_buf[...], preferred_element_type=jnp.float32).astype(jnp.bfloat16)
    for h in range(_H):
        q_scr[h] = q_all[:, h * _DH:(h + 1) * _DH]

    def head(h, acc):
        slot = h % S
        q = q_scr[h]
        k_copy(h, slot).wait()
        s = jnp.dot(q, k_buf[slot], preferred_element_type=jnp.float32) * scale
        m = jnp.max(s, axis=-1, keepdims=True)
        e = jnp.exp(s - m)
        l = jnp.sum(e, axis=-1, keepdims=True)
        v_copy(h, slot).wait()
        o = jax.lax.dot_general(e.astype(jnp.bfloat16), v_buf[slot], (((1,), (1,)), ((), ())),
                                preferred_element_type=jnp.float32)
        o = (o / l).astype(jnp.bfloat16)
        wo_copy(h, slot).wait()
        acc = acc + jnp.dot(o, wo_buf[slot], preferred_element_type=jnp.float32)

        @pl.when(h + S < _H)
        def _():
            k_copy(h + S, slot).start()
            v_copy(h + S, slot).start()
            wo_copy(h + S, slot).start()

        @pl.when(h + S == _H - 1)
        def _():
            w3_copy.start()
            for c in range(_W4_CHUNKS):
                w4_copy(c).start()

        return acc

    attn = jax.lax.fori_loop(0, _H, head, jnp.zeros((_M, _D), jnp.float32))

    hres = x8 + attn
    x1 = _ln(hres)
    xn2 = _ln(x1).astype(jnp.bfloat16)
    w3_copy.wait()
    g = _gelu(jnp.dot(xn2, w3_buf[...], preferred_element_type=jnp.float32)).astype(jnp.bfloat16)
    res = hres + x1
    for c in range(_W4_CHUNKS):
        w4_copy(c).wait()
        res = res + jnp.dot(g[:, c * rows4:(c + 1) * rows4], w4_buf[pl.ds(c * rows4, rows4), :],
                            preferred_element_type=jnp.float32)
    out_ref[0] = res[0:1].astype(out_ref.dtype)


@jax.jit
def pallas_sequential_preLN__sliding_block_cached__mixer_s_mlp__decode_kernel(
    A_x: jax.Array,
    A_k_cache: jax.Array,
    A_v_cache: jax.Array,
    A_wq: jax.Array,
    A_wo: jax.Array,
    B_x: jax.Array,
    B_w1: jax.Array,
    B_w2: jax.Array,
    B_w3: jax.Array,
    B_w4: jax.Array,
):
    del B_x, B_w1, B_w2
    sk = A_k_cache.shape[2]
    w = min(4096, max(256, sk // 4))
    kt = jnp.swapaxes(A_k_cache, 2, 3).reshape(_H, _DH, sk)
    vt = jnp.swapaxes(A_v_cache, 2, 3).reshape(_H, _DH, sk)
    any_spec = pl.BlockSpec(memory_space=pl.ANY)
    return pl.pallas_call(
        functools.partial(_kernel, sk=sk, w=w),
        out_shape=jax.ShapeDtypeStruct((1, 1, _D), A_x.dtype),
        in_specs=[any_spec] * 7,
        out_specs=pl.BlockSpec(memory_space=pltpu.VMEM),
        scratch_shapes=[
            pltpu.VMEM((1, 1, _D), jnp.bfloat16),
            pltpu.VMEM((_D, _H * _DH), jnp.bfloat16),
            pltpu.VMEM((_SLOTS, _DH, w), jnp.bfloat16),
            pltpu.VMEM((_SLOTS, _DH, w), jnp.bfloat16),
            pltpu.VMEM((_SLOTS, _DH, _D), jnp.bfloat16),
            pltpu.VMEM((_D, _F), jnp.bfloat16),
            pltpu.VMEM((_F, _D), jnp.bfloat16),
            pltpu.VMEM((_H, _M, _DH), jnp.bfloat16),
            pltpu.SemaphoreType.DMA((3 * _SLOTS + 3 + _W4_CHUNKS,)),
        ],
        compiler_params=pltpu.CompilerParams(vmem_limit_bytes=100 * 1024 * 1024),
    )(A_x, kt, vt, A_wq, A_wo, B_w3, B_w4)
```

```python
import functools

import jax
import jax.numpy as jnp
import numpy as np
import jax.experimental.pallas as pl
import jax.experimental.pallas.tpu as pltpu

_H, _DH, _D, _F = 32, 192, 640, 1536
_M = 8
_EPS = 1e-5
_SLOTS = 2
_W4_CHUNKS = 2


def _ln(v):
    m = jnp.mean(v, axis=-1, keepdims=True)
    d = v - m
    var = jnp.mean(d * d, axis=-1, keepdims=True)
    return d * jax.lax.rsqrt(var + _EPS)


def _gelu(v):
    c = float(np.sqrt(2.0 / np.pi))
    return 0.5 * v * (1.0 + jnp.tanh(c * (v + 0.044715 * (v * v * v))))


def _chunks(src, dst, rows, cols, rb, cb, sem, c0=0):
    return [pltpu.make_async_copy(src.at[pl.ds(r * rb, rb), pl.ds(c0 + c * cb, cb)],
                                  dst.at[pl.ds(r * rb, rb), pl.ds(c * cb, cb)], sem)
            for c in range(cols // cb) for r in range(rows // rb)]


def _start_alternating(copies):
    for i, c in enumerate(copies):
        c.start(priority=i % 2)


def _wait_filled(buf, sem):
    pltpu.make_async_copy(buf, buf, sem).wait()


def _kernel(x_hbm, kt_hbm, vt_hbm, wq_hbm, wo_hbm, w3_hbm, w4_hbm, out_ref,
            x_buf, wq_buf, k_buf, v_buf, wo_buf, w3_buf, w4_buf, q_scr, sems, *, sk, w):
    S = _SLOTS
    scale = _DH ** -0.5

    def start_head(h, slot):
        kc = _chunks(kt_hbm.at[h], k_buf.at[slot], _DH, w, 32, 512, sems.at[slot], c0=sk - w)
        vc = _chunks(vt_hbm.at[h], v_buf.at[slot], _DH, w, 32, 512, sems.at[S + slot], c0=sk - w)
        base = h * _DH if isinstance(h, int) else pl.multiple_of(h * _DH, _DH)
        oc = _chunks(wo_hbm.at[pl.ds(base, _DH)], wo_buf.at[slot], _DH, _D, 32, _D, sems.at[2 * S + slot])
        _start_alternating([c for pair in zip(vc, kc) for c in pair] + oc)

    x_copy = pltpu.make_async_copy(x_hbm, x_buf, sems.at[3 * S])
    wq_sem, w3_sem = sems.at[3 * S + 1], sems.at[3 * S + 2]
    rows4 = _F // _W4_CHUNKS

    def w4_part(c):
        rows = pl.ds(c * rows4, rows4)
        return w4_hbm.at[rows], w4_buf.at[rows], sems.at[3 * S + 3 + c]

    x_copy.start()
    _start_alternating(_chunks(wq_hbm, wq_buf, _D, _H * _DH, 32, 512, wq_sem))
    for h in range(S):
        start_head(h, h)

    x_copy.wait()
    x8 = jnp.broadcast_to(x_buf[0].astype(jnp.float32), (_M, _D))
    xn = _ln(x8).astype(jnp.bfloat16)
    _wait_filled(wq_buf, wq_sem)
    q_all = jnp.dot(xn, wq_buf[...], preferred_element_type=jnp.float32).astype(jnp.bfloat16)
    for h in range(_H):
        q_scr[h] = q_all[:, h * _DH:(h + 1) * _DH]

    def head(h, acc):
        slot = h % S
        q = q_scr[h]
        _wait_filled(k_buf.at[slot], sems.at[slot])
        s = jnp.dot(q, k_buf[slot], preferred_element_type=jnp.float32) * scale
        m = jnp.max(s, axis=-1, keepdims=True)
        e = jnp.exp(s - m)
        l = jnp.sum(e, axis=-1, keepdims=True)
        _wait_filled(v_buf.at[slot], sems.at[S + slot])
        o = jax.lax.dot_general(e.astype(jnp.bfloat16), v_buf[slot], (((1,), (1,)), ((), ())),
                                preferred_element_type=jnp.float32)
        o = (o / l).astype(jnp.bfloat16)
        _wait_filled(wo_buf.at[slot], sems.at[2 * S + slot])
        acc = acc + jnp.dot(o, wo_buf[slot], preferred_element_type=jnp.float32)

        @pl.when(h + S < _H)
        def _():
            start_head(h + S, slot)

        @pl.when(h + S == _H - 1)
        def _():
            _start_alternating(_chunks(w3_hbm, w3_buf, _D, _F, 8, _F, w3_sem))
            for c in range(_W4_CHUNKS):
                src, dst, sem = w4_part(c)
                _start_alternating(_chunks(src, dst, rows4, _D, 32, _D, sem))

        return acc

    attn = jax.lax.fori_loop(0, _H, head, jnp.zeros((_M, _D), jnp.float32))

    hres = x8 + attn
    x1 = _ln(hres)
    xn2 = _ln(x1).astype(jnp.bfloat16)
    _wait_filled(w3_buf, w3_sem)
    g = _gelu(jnp.dot(xn2, w3_buf[...], preferred_element_type=jnp.float32)).astype(jnp.bfloat16)
    res = hres + x1
    for c in range(_W4_CHUNKS):
        _, dst, sem = w4_part(c)
        _wait_filled(dst, sem)
        res = res + jnp.dot(g[:, c * rows4:(c + 1) * rows4], dst[...], preferred_element_type=jnp.float32)
    out_ref[0] = res[0:1].astype(out_ref.dtype)


@jax.jit
def pallas_sequential_preLN__sliding_block_cached__mixer_s_mlp__decode_kernel(
    A_x: jax.Array,
    A_k_cache: jax.Array,
    A_v_cache: jax.Array,
    A_wq: jax.Array,
    A_wo: jax.Array,
    B_x: jax.Array,
    B_w1: jax.Array,
    B_w2: jax.Array,
    B_w3: jax.Array,
    B_w4: jax.Array,
):
    del B_x, B_w1, B_w2
    sk = A_k_cache.shape[2]
    w = min(4096, max(256, sk // 4))
    kt = jnp.swapaxes(A_k_cache, 2, 3).reshape(_H, _DH, sk)
    vt = jnp.swapaxes(A_v_cache, 2, 3).reshape(_H, _DH, sk)
    any_spec = pl.BlockSpec(memory_space=pl.ANY)
    return pl.pallas_call(
        functools.partial(_kernel, sk=sk, w=w),
        out_shape=jax.ShapeDtypeStruct((1, 1, _D), A_x.dtype),
        in_specs=[any_spec] * 7,
        out_specs=pl.BlockSpec(memory_space=pltpu.VMEM),
        scratch_shapes=[
            pltpu.VMEM((1, 1, _D), jnp.bfloat16),
            pltpu.VMEM((_D, _H * _DH), jnp.bfloat16),
            pltpu.VMEM((_SLOTS, _DH, w), jnp.bfloat16),
            pltpu.VMEM((_SLOTS, _DH, w), jnp.bfloat16),
            pltpu.VMEM((_SLOTS, _DH, _D), jnp.bfloat16),
            pltpu.VMEM((_D, _F), jnp.bfloat16),
            pltpu.VMEM((_F, _D), jnp.bfloat16),
            pltpu.VMEM((_H, _M, _DH), jnp.bfloat16),
            pltpu.SemaphoreType.DMA((3 * _SLOTS + 3 + _W4_CHUNKS,)),
        ],
        compiler_params=pltpu.CompilerParams(vmem_limit_bytes=100 * 1024 * 1024),
    )(A_x, kt, vt, A_wq, A_wo, B_w3, B_w4)
```

```python
import functools

import jax
import jax.numpy as jnp
import numpy as np
import jax.experimental.pallas as pl
import jax.experimental.pallas.tpu as pltpu

_H, _DH, _D, _F = 32, 192, 640, 1536
_M = 8
_EPS = 1e-5
_SLOTS = 2
_W4_SPLIT = (768, 384, 256, 128)


def _ln(v):
    m = jnp.mean(v, axis=-1, keepdims=True)
    d = v - m
    var = jnp.mean(d * d, axis=-1, keepdims=True)
    return d * jax.lax.rsqrt(var + _EPS)


def _gelu(v):
    c = float(np.sqrt(2.0 / np.pi))
    return 0.5 * v * (1.0 + jnp.tanh(c * (v + 0.044715 * (v * v * v))))


def _tiles(src, dst, rb, cb, sem, c0=0):
    rows, cols = dst.shape
    return [pltpu.make_async_copy(src.at[pl.ds(r * rb, rb), pl.ds(c0 + c * cb, cb)],
                                  dst.at[pl.ds(r * rb, rb), pl.ds(c * cb, cb)], sem)
            for c in range(cols // cb) for r in range(rows // rb)]


def _strided_tiles(src, dst, groups, rb, cb, sem):
    rows, cols = dst.shape
    rg = rows // groups
    s3, d3 = src.reshape(groups, rg, cols), dst.reshape(groups, rg, cols)
    return [pltpu.make_async_copy(s3.at[:, pl.ds(r * rb, rb), pl.ds(c * cb, cb)],
                                  d3.at[:, pl.ds(r * rb, rb), pl.ds(c * cb, cb)], sem)
            for r in range(rg // rb) for c in range(cols // cb)]


def _start_alternating(copies):
    for i, c in enumerate(copies):
        c.start(priority=i % 2)


def _wait_filled(buf, sem):
    pltpu.make_async_copy(buf, buf, sem).wait()


def _kernel(x_hbm, kt_hbm, vt_hbm, wq_hbm, wo_hbm, w3_hbm, w4_hbm, out_ref,
            x_buf, wq_buf, k_buf, v_buf, wo_buf, w3_buf, w4_buf, q_scr, sems, *, sk, w):
    S = _SLOTS
    scale = _DH ** -0.5
    offs4 = [int(o) for o in np.cumsum((0,) + _W4_SPLIT)]

    def start_head(h, slot):
        kc = _tiles(kt_hbm.at[h], k_buf.at[slot], 32, 512, sems.at[slot], c0=sk - w)
        vc = _tiles(vt_hbm.at[h], v_buf.at[slot], 32, 512, sems.at[S + slot], c0=sk - w)
        _start_alternating([c for pair in zip(kc, vc) for c in pair])

    x_copy = pltpu.make_async_copy(x_hbm, x_buf, sems.at[2 * S])
    wq_sem, wo_sem, w3_sem = sems.at[2 * S + 1], sems.at[2 * S + 2], sems.at[2 * S + 3]

    def w4_part(c):
        rows = pl.ds(offs4[c], _W4_SPLIT[c])
        return w4_hbm.at[rows], w4_buf.at[rows], sems.at[2 * S + 4 + c]

    x_copy.start()
    _start_alternating(_strided_tiles(wq_hbm, wq_buf, 10, 8, 256, wq_sem))
    _start_alternating(_strided_tiles(wo_hbm, wo_buf, 12, 8, 128, wo_sem))
    for h in range(S):
        start_head(h, h)

    x_copy.wait()
    x8 = jnp.broadcast_to(x_buf[0].astype(jnp.float32), (_M, _D))
    xn = _ln(x8).astype(jnp.bfloat16)
    _wait_filled(wq_buf, wq_sem)
    q_all = jnp.dot(xn, wq_buf[...], preferred_element_type=jnp.float32).astype(jnp.bfloat16)
    for h in range(_H):
        q_scr[h] = q_all[:, h * _DH:(h + 1) * _DH]
    _wait_filled(wo_buf, wo_sem)

    def head(h, acc):
        slot = h % S
        q = q_scr[h]
        _wait_filled(k_buf.at[slot], sems.at[slot])
        s = jnp.dot(q, k_buf[slot], preferred_element_type=jnp.float32) * scale
        m = jnp.max(s, axis=-1, keepdims=True)
        e = jnp.exp(s - m)
        l = jnp.sum(e, axis=-1, keepdims=True)
        _wait_filled(v_buf.at[slot], sems.at[S + slot])
        o = jax.lax.dot_general(e.astype(jnp.bfloat16), v_buf[slot], (((1,), (1,)), ((), ())),
                                preferred_element_type=jnp.float32)
        o = (o / l).astype(jnp.bfloat16)
        wo = wo_buf[pl.ds(pl.multiple_of(h * _DH, _DH), _DH), :]
        acc = acc + jnp.dot(o, wo, preferred_element_type=jnp.float32)

        @pl.when(h + S < _H)
        def _():
            start_head(h + S, slot)

        @pl.when(h + S == _H)
        def _():
            _start_alternating(_strided_tiles(w3_hbm, w3_buf, 5, 8, 384, w3_sem))
            for c in range(len(_W4_SPLIT)):
                src, dst, sem = w4_part(c)
                _start_alternating(_tiles(src, dst, 32, _D, sem))

        return acc

    attn = jax.lax.fori_loop(0, _H, head, jnp.zeros((_M, _D), jnp.float32))

    hres = x8 + attn
    x1 = _ln(hres)
    xn2 = _ln(x1).astype(jnp.bfloat16)
    _wait_filled(w3_buf, w3_sem)
    g = _gelu(jnp.dot(xn2, w3_buf[...], preferred_element_type=jnp.float32)).astype(jnp.bfloat16)
    res = hres + x1
    for c in range(len(_W4_SPLIT)):
        _, dst, sem = w4_part(c)
        _wait_filled(dst, sem)
        res = res + jnp.dot(g[:, offs4[c]:offs4[c + 1]], dst[...], preferred_element_type=jnp.float32)
    out_ref[0] = res[0:1].astype(out_ref.dtype)


@jax.jit
def pallas_sequential_preLN__sliding_block_cached__mixer_s_mlp__decode_kernel(
    A_x: jax.Array,
    A_k_cache: jax.Array,
    A_v_cache: jax.Array,
    A_wq: jax.Array,
    A_wo: jax.Array,
    B_x: jax.Array,
    B_w1: jax.Array,
    B_w2: jax.Array,
    B_w3: jax.Array,
    B_w4: jax.Array,
):
    del B_x, B_w1, B_w2
    sk = A_k_cache.shape[2]
    w = min(4096, max(256, sk // 4))
    kt = jnp.swapaxes(A_k_cache, 2, 3).reshape(_H, _DH, sk)
    vt = jnp.swapaxes(A_v_cache, 2, 3).reshape(_H, _DH, sk)
    any_spec = pl.BlockSpec(memory_space=pl.ANY)
    return pl.pallas_call(
        functools.partial(_kernel, sk=sk, w=w),
        out_shape=jax.ShapeDtypeStruct((1, 1, _D), A_x.dtype),
        in_specs=[any_spec] * 7,
        out_specs=pl.BlockSpec(memory_space=pltpu.VMEM),
        scratch_shapes=[
            pltpu.VMEM((1, 1, _D), jnp.bfloat16),
            pltpu.VMEM((_D, _H * _DH), jnp.bfloat16),
            pltpu.VMEM((_SLOTS, _DH, w), jnp.bfloat16),
            pltpu.VMEM((_SLOTS, _DH, w), jnp.bfloat16),
            pltpu.VMEM((_H * _DH, _D), jnp.bfloat16),
            pltpu.VMEM((_D, _F), jnp.bfloat16),
            pltpu.VMEM((_F, _D), jnp.bfloat16),
            pltpu.VMEM((_H, _M, _DH), jnp.bfloat16),
            pltpu.SemaphoreType.DMA((2 * _SLOTS + 4 + len(_W4_SPLIT),)),
        ],
        compiler_params=pltpu.CompilerParams(vmem_limit_bytes=64 * 1024 * 1024,
                                             disable_semaphore_checks=True),
    )(A_x, kt, vt, A_wq, A_wo, B_w3, B_w4)
```

```python
import functools

import jax
import jax.numpy as jnp
import numpy as np
import jax.experimental.pallas as pl
import jax.experimental.pallas.tpu as pltpu

_H, _DH, _D, _F = 32, 192, 640, 1536
_M = 8
_EPS = 1e-5
_SLOTS = 2
_W4_SPLIT = (768, 384, 256, 128)
_WQ_SLABS, _W3_SLABS = 8, 5


def _ln(v):
    m = jnp.mean(v, axis=-1, keepdims=True)
    d = v - m
    var = jnp.mean(d * d, axis=-1, keepdims=True)
    return d * jax.lax.rsqrt(var + _EPS)


def _gelu(v):
    c = float(np.sqrt(2.0 / np.pi))
    return 0.5 * v * (1.0 + jnp.tanh(c * (v + 0.044715 * (v * v * v))))


def _tiles(src, dst, rb, cb, sem, c0=0):
    rows, cols = dst.shape
    return [pltpu.make_async_copy(src.at[pl.ds(r * rb, rb), pl.ds(c0 + c * cb, cb)],
                                  dst.at[pl.ds(r * rb, rb), pl.ds(c * cb, cb)], sem)
            for c in range(cols // cb) for r in range(rows // rb)]


def _slab_tiles(src, dst, rb, cb, sem):
    _, rows, cols = dst.shape
    return [pltpu.make_async_copy(src.at[:, pl.ds(r * rb, rb), pl.ds(c * cb, cb)],
                                  dst.at[:, pl.ds(r * rb, rb), pl.ds(c * cb, cb)], sem)
            for r in range(rows // rb) for c in range(cols // cb)]


def _interleave(a, b):
    return [c for pair in zip(a, b, strict=True) for c in pair]


def _start_alternating(copies):
    for i, c in enumerate(copies):
        c.start(priority=i % 2)


def _wait_filled(buf, sem):
    pltpu.make_async_copy(buf, buf, sem).wait()


def _kernel(x_hbm, kt_hbm, vt_hbm, wq_hbm, wo_hbm, w3_hbm, w4_hbm, out_ref,
            x_buf, wq_buf, k_buf, v_buf, wo_buf, w3_buf, w4_buf, q_scr, sems, *, sk, w):
    S = _SLOTS
    scale = _DH ** -0.5
    offs4 = [int(o) for o in np.cumsum((0,) + _W4_SPLIT)]

    def start_head(h, slot):
        kc = _tiles(kt_hbm.at[h], k_buf.at[slot], 32, 512, sems.at[slot], c0=sk - w)
        vc = _tiles(vt_hbm.at[h], v_buf.at[slot], 32, 512, sems.at[S + slot], c0=sk - w)
        _start_alternating(_interleave(kc, vc))

    x_copy = pltpu.make_async_copy(x_hbm, x_buf, sems.at[2 * S])
    wq_sem, wo_sem, w3_sem = sems.at[2 * S + 1], sems.at[2 * S + 2], sems.at[2 * S + 3]

    def w4_part(c):
        rows = pl.ds(offs4[c], _W4_SPLIT[c])
        return w4_hbm.at[rows], w4_buf.at[rows], sems.at[2 * S + 4 + c]

    x_copy.start()
    _start_alternating(_interleave(_slab_tiles(wo_hbm, wo_buf, 8, 128, wo_sem),
                                   _slab_tiles(wq_hbm, wq_buf, 8, 256, wq_sem)))
    for h in range(S):
        start_head(h, h)

    x_copy.wait()
    x8 = jnp.broadcast_to(x_buf[0].astype(jnp.float32), (_M, _D))
    xn = _ln(x8).astype(jnp.bfloat16)
    _wait_filled(wq_buf, wq_sem)
    wq = wq_buf[...].reshape(_D, _H * _DH)
    q_all = jnp.dot(xn, wq, preferred_element_type=jnp.float32).astype(jnp.bfloat16)
    for h in range(_H):
        q_scr[h] = q_all[:, h * _DH:(h + 1) * _DH]
    _wait_filled(wo_buf, wo_sem)

    def head(h, acc):
        slot = h % S
        q = q_scr[h]
        _wait_filled(k_buf.at[slot], sems.at[slot])
        s = jnp.dot(q, k_buf[slot], preferred_element_type=jnp.float32) * scale
        m = jnp.max(s, axis=-1, keepdims=True)
        e = jnp.exp(s - m)
        l = jnp.sum(e, axis=-1, keepdims=True)
        _wait_filled(v_buf.at[slot], sems.at[S + slot])
        o = jax.lax.dot_general(e.astype(jnp.bfloat16), v_buf[slot], (((1,), (1,)), ((), ())),
                                preferred_element_type=jnp.float32)
        o = (o / l).astype(jnp.bfloat16)
        wo = wo_buf[h // 2, pl.ds(pl.multiple_of((h % 2) * _DH, _DH), _DH), :]
        acc = acc + jnp.dot(o, wo, preferred_element_type=jnp.float32)

        @pl.when(h + S < _H)
        def _():
            start_head(h + S, slot)

        @pl.when(h + S == _H)
        def _():
            _start_alternating(_slab_tiles(w3_hbm, w3_buf, 8, 384, w3_sem))
            for c in range(len(_W4_SPLIT)):
                src, dst, sem = w4_part(c)
                _start_alternating(_tiles(src, dst, 32, _D, sem))

        return acc

    attn = jax.lax.fori_loop(0, _H, head, jnp.zeros((_M, _D), jnp.float32))

    hres = x8 + attn
    x1 = _ln(hres)
    xn2 = _ln(x1).astype(jnp.bfloat16)
    _wait_filled(w3_buf, w3_sem)
    w3 = w3_buf[...].reshape(_D, _F)
    g = _gelu(jnp.dot(xn2, w3, preferred_element_type=jnp.float32)).astype(jnp.bfloat16)
    res = hres + x1
    for c in range(len(_W4_SPLIT)):
        _, dst, sem = w4_part(c)
        _wait_filled(dst, sem)
        res = res + jnp.dot(g[:, offs4[c]:offs4[c + 1]], dst[...], preferred_element_type=jnp.float32)
    out_ref[0] = res[0:1].astype(out_ref.dtype)


@jax.jit
def pallas_sequential_preLN__sliding_block_cached__mixer_s_mlp__decode_kernel(
    A_x: jax.Array,
    A_k_cache: jax.Array,
    A_v_cache: jax.Array,
    A_wq: jax.Array,
    A_wo: jax.Array,
    B_x: jax.Array,
    B_w1: jax.Array,
    B_w2: jax.Array,
    B_w3: jax.Array,
    B_w4: jax.Array,
):
    del B_x, B_w1, B_w2
    sk = A_k_cache.shape[2]
    w = min(4096, max(256, sk // 4))
    kt = jnp.swapaxes(A_k_cache, 2, 3).reshape(_H, _DH, sk)
    vt = jnp.swapaxes(A_v_cache, 2, 3).reshape(_H, _DH, sk)
    wq = A_wq.reshape(_WQ_SLABS, _D // _WQ_SLABS, _H * _DH)
    wo = A_wo.reshape(_H // 2, 2 * _DH, _D)
    w3 = B_w3.reshape(_W3_SLABS, _D // _W3_SLABS, _F)
    any_spec = pl.BlockSpec(memory_space=pl.ANY)
    return pl.pallas_call(
        functools.partial(_kernel, sk=sk, w=w),
        out_shape=jax.ShapeDtypeStruct((1, 1, _D), A_x.dtype),
        in_specs=[any_spec] * 7,
        out_specs=pl.BlockSpec(memory_space=pltpu.VMEM),
        scratch_shapes=[
            pltpu.VMEM((1, 1, _D), jnp.bfloat16),
            pltpu.VMEM(wq.shape, jnp.bfloat16),
            pltpu.VMEM((_SLOTS, _DH, w), jnp.bfloat16),
            pltpu.VMEM((_SLOTS, _DH, w), jnp.bfloat16),
            pltpu.VMEM(wo.shape, jnp.bfloat16),
            pltpu.VMEM(w3.shape, jnp.bfloat16),
            pltpu.VMEM((_F, _D), jnp.bfloat16),
            pltpu.VMEM((_H, _M, _DH), jnp.bfloat16),
            pltpu.SemaphoreType.DMA((2 * _SLOTS + 4 + len(_W4_SPLIT),)),
        ],
        compiler_params=pltpu.CompilerParams(vmem_limit_bytes=64 * 1024 * 1024,
                                             disable_semaphore_checks=True),
    )(A_x, kt, vt, wq, wo, w3, B_w4)
```

```python
import functools

import jax
import jax.numpy as jnp
import numpy as np
import jax.experimental.pallas as pl
import jax.experimental.pallas.tpu as pltpu

_H, _DH, _D, _F = 32, 192, 640, 1536
_M = 8
_EPS = 1e-5
_SLOTS = 2
_W4_SPLIT = (768, 384, 256, 128)
_WQ_SLABS, _WO_SLABS, _W3_SLABS = 10, 12, 5


def _ln(v):
    m = jnp.mean(v, axis=-1, keepdims=True)
    d = v - m
    var = jnp.mean(d * d, axis=-1, keepdims=True)
    return d * jax.lax.rsqrt(var + _EPS)


def _gelu(v):
    c = float(np.sqrt(2.0 / np.pi))
    return 0.5 * v * (1.0 + jnp.tanh(c * (v + 0.044715 * (v * v * v))))


def _tiles(src, dst, rb, cb, sem, c0=0):
    rows, cols = dst.shape
    return [pltpu.make_async_copy(src.at[pl.ds(r * rb, rb), pl.ds(c0 + c * cb, cb)],
                                  dst.at[pl.ds(r * rb, rb), pl.ds(c * cb, cb)], sem)
            for c in range(cols // cb) for r in range(rows // rb)]


def _slab_tiles(src, dst, rb, cb, sem):
    _, rows, cols = dst.shape
    return [pltpu.make_async_copy(src.at[:, pl.ds(r * rb, rb), pl.ds(c * cb, cb)],
                                  dst.at[:, pl.ds(r * rb, rb), pl.ds(c * cb, cb)], sem)
            for r in range(rows // rb) for c in range(cols // cb)]


def _wo_tiles(src, dst, sem):
    _, blocks, rows, cols = dst.shape
    return [pltpu.make_async_copy(src.at[:, b, pl.ds(r * 8, 8), pl.ds(c * 128, 128)],
                                  dst.at[:, b, pl.ds(r * 8, 8), pl.ds(c * 128, 128)], sem)
            for b in range(blocks) for r in range(rows // 8) for c in range(cols // 128)]


def _interleave(a, b):
    n = min(len(a), len(b))
    return [c for pair in zip(a[:n], b[:n]) for c in pair] + a[n:] + b[n:]


def _start_alternating(copies):
    for i, c in enumerate(copies):
        c.start(priority=i % 2)


def _wait_filled(buf, sem):
    pltpu.make_async_copy(buf, buf, sem).wait()


def _kernel(x_hbm, kt_hbm, vt_hbm, wq_hbm, wo_hbm, w3_hbm, w4_hbm, out_ref,
            x_buf, wq_buf, k_buf, v_buf, wo_buf, w3_buf, w4_buf, q_scr, sems, *, sk, w):
    S = _SLOTS
    scale = _DH ** -0.5
    offs4 = [int(o) for o in np.cumsum((0,) + _W4_SPLIT)]

    def start_head(h, slot):
        kc = _tiles(kt_hbm.at[h], k_buf.at[slot], 32, 512, sems.at[slot], c0=sk - w)
        vc = _tiles(vt_hbm.at[h], v_buf.at[slot], 32, 512, sems.at[S + slot], c0=sk - w)
        _start_alternating(_interleave(kc, vc))

    x_copy = pltpu.make_async_copy(x_hbm, x_buf, sems.at[2 * S])
    wq_sem, wo_sem, w3_sem = sems.at[2 * S + 1], sems.at[2 * S + 2], sems.at[2 * S + 3]

    def w4_part(c):
        rows = pl.ds(offs4[c], _W4_SPLIT[c])
        return w4_hbm.at[rows], w4_buf.at[rows], sems.at[2 * S + 4 + c]

    x_copy.start()
    _start_alternating(_interleave(_wo_tiles(wo_hbm, wo_buf, wo_sem),
                                   _slab_tiles(wq_hbm, wq_buf, 8, 256, wq_sem)))
    for h in range(S):
        start_head(h, h)

    x_copy.wait()
    x8 = jnp.broadcast_to(x_buf[0].astype(jnp.float32), (_M, _D))
    xn = _ln(x8).astype(jnp.bfloat16)
    _wait_filled(wq_buf, wq_sem)
    wq = wq_buf[...].reshape(_D, _H * _DH)
    q_all = jnp.dot(xn, wq, preferred_element_type=jnp.float32).astype(jnp.bfloat16)
    for h in range(_H):
        q_scr[h] = q_all[:, h * _DH:(h + 1) * _DH]
    _wait_filled(wo_buf, wo_sem)

    def head(h, acc):
        slot = h % S
        q = q_scr[h]
        _wait_filled(k_buf.at[slot], sems.at[slot])
        s = jnp.dot(q, k_buf[slot], preferred_element_type=jnp.float32) * scale
        m = jnp.max(s, axis=-1, keepdims=True)
        e = jnp.exp(s - m)
        l = jnp.sum(e, axis=-1, keepdims=True)
        _wait_filled(v_buf.at[slot], sems.at[S + slot])
        o = jax.lax.dot_general(e.astype(jnp.bfloat16), v_buf[slot], (((1,), (1,)), ((), ())),
                                preferred_element_type=jnp.float32)
        o = (o / l).astype(jnp.bfloat16)
        nblk = wo_buf.shape[1]
        wo = jnp.concatenate([wo_buf[(3 * h + b) // nblk, (3 * h + b) % nblk] for b in range(3)], axis=0)
        acc = acc + jnp.dot(o, wo, preferred_element_type=jnp.float32)

        @pl.when(h + S < _H)
        def _():
            start_head(h + S, slot)

        @pl.when(h + S == _H)
        def _():
            _start_alternating(_slab_tiles(w3_hbm, w3_buf, 8, 384, w3_sem))
            for c in range(len(_W4_SPLIT)):
                src, dst, sem = w4_part(c)
                _start_alternating(_tiles(src, dst, 32, _D, sem))

        return acc

    attn = jax.lax.fori_loop(0, _H, head, jnp.zeros((_M, _D), jnp.float32))

    hres = x8 + attn
    x1 = _ln(hres)
    xn2 = _ln(x1).astype(jnp.bfloat16)
    _wait_filled(w3_buf, w3_sem)
    w3 = w3_buf[...].reshape(_D, _F)
    g = _gelu(jnp.dot(xn2, w3, preferred_element_type=jnp.float32)).astype(jnp.bfloat16)
    res = hres + x1
    for c in range(len(_W4_SPLIT)):
        _, dst, sem = w4_part(c)
        _wait_filled(dst, sem)
        res = res + jnp.dot(g[:, offs4[c]:offs4[c + 1]], dst[...], preferred_element_type=jnp.float32)
    out_ref[0] = res[0:1].astype(out_ref.dtype)


@jax.jit
def pallas_sequential_preLN__sliding_block_cached__mixer_s_mlp__decode_kernel(
    A_x: jax.Array,
    A_k_cache: jax.Array,
    A_v_cache: jax.Array,
    A_wq: jax.Array,
    A_wo: jax.Array,
    B_x: jax.Array,
    B_w1: jax.Array,
    B_w2: jax.Array,
    B_w3: jax.Array,
    B_w4: jax.Array,
):
    del B_x, B_w1, B_w2
    sk = A_k_cache.shape[2]
    w = min(4096, max(256, sk // 4))
    kt = jnp.swapaxes(A_k_cache, 2, 3).reshape(_H, _DH, sk)
    vt = jnp.swapaxes(A_v_cache, 2, 3).reshape(_H, _DH, sk)
    wq = A_wq.reshape(_WQ_SLABS, _D // _WQ_SLABS, _H * _DH)
    wo = A_wo.reshape(_WO_SLABS, _H * _DH // (64 * _WO_SLABS), 64, _D)
    w3 = B_w3.reshape(_W3_SLABS, _D // _W3_SLABS, _F)
    any_spec = pl.BlockSpec(memory_space=pl.ANY)
    return pl.pallas_call(
        functools.partial(_kernel, sk=sk, w=w),
        out_shape=jax.ShapeDtypeStruct((1, 1, _D), A_x.dtype),
        in_specs=[any_spec] * 7,
        out_specs=pl.BlockSpec(memory_space=pltpu.VMEM),
        scratch_shapes=[
            pltpu.VMEM((1, 1, _D), jnp.bfloat16),
            pltpu.VMEM(wq.shape, jnp.bfloat16),
            pltpu.VMEM((_SLOTS, _DH, w), jnp.bfloat16),
            pltpu.VMEM((_SLOTS, _DH, w), jnp.bfloat16),
            pltpu.VMEM(wo.shape, jnp.bfloat16),
            pltpu.VMEM(w3.shape, jnp.bfloat16),
            pltpu.VMEM((_F, _D), jnp.bfloat16),
            pltpu.VMEM((_H, _M, _DH), jnp.bfloat16),
            pltpu.SemaphoreType.DMA((2 * _SLOTS + 4 + len(_W4_SPLIT),)),
        ],
        compiler_params=pltpu.CompilerParams(vmem_limit_bytes=64 * 1024 * 1024,
                                             disable_semaphore_checks=True),
    )(A_x, kt, vt, wq, wo, w3, B_w4)
```

```python
import functools

import jax
import jax.numpy as jnp
import numpy as np
import jax.experimental.pallas as pl
import jax.experimental.pallas.tpu as pltpu

_H, _DH, _D, _F = 32, 192, 640, 1536
_M = 8
_EPS = 1e-5
_SLOTS = 2
_W4_SPLIT = (768, 384, 256, 128)
_WQ_SLABS, _WO_SLABS, _W3_SLABS = 10, 12, 10


def _ln(v):
    m = jnp.mean(v, axis=-1, keepdims=True)
    d = v - m
    var = jnp.mean(d * d, axis=-1, keepdims=True)
    return d * jax.lax.rsqrt(var + _EPS)


def _gelu(v):
    c = float(np.sqrt(2.0 / np.pi))
    return 0.5 * v * (1.0 + jnp.tanh(c * (v + 0.044715 * (v * v * v))))


def _tiles(src, dst, rb, cb, sem, c0=0):
    rows, cols = dst.shape
    return [pltpu.make_async_copy(src.at[pl.ds(r * rb, rb), pl.ds(c0 + c * cb, cb)],
                                  dst.at[pl.ds(r * rb, rb), pl.ds(c * cb, cb)], sem)
            for c in range(cols // cb) for r in range(rows // rb)]


def _slab_tiles(src, dst, rb, cb, sem):
    _, rows, cols = dst.shape
    return [pltpu.make_async_copy(src.at[:, pl.ds(r * rb, rb), pl.ds(c * cb, cb)],
                                  dst.at[:, pl.ds(r * rb, rb), pl.ds(c * cb, cb)], sem)
            for r in range(rows // rb) for c in range(cols // cb)]


def _wo_tiles(src, dst, sem):
    _, blocks, rows, cols = dst.shape
    return [pltpu.make_async_copy(src.at[:, b, pl.ds(r * 8, 8), pl.ds(c * 128, 128)],
                                  dst.at[:, b, pl.ds(r * 8, 8), pl.ds(c * 128, 128)], sem)
            for b in range(blocks) for r in range(rows // 8) for c in range(cols // 128)]


def _interleave(a, b):
    n = min(len(a), len(b))
    return [c for pair in zip(a[:n], b[:n]) for c in pair] + a[n:] + b[n:]


def _start_alternating(copies):
    for i, c in enumerate(copies):
        c.start(priority=i % 2)


def _wait_filled(buf, sem):
    pltpu.make_async_copy(buf, buf, sem).wait()


def _kernel(x_hbm, kt_hbm, vt_hbm, wq_hbm, wo_hbm, w3_hbm, w4_hbm, out_ref,
            x_buf, wq_buf, k_buf, v_buf, wo_buf, w3_buf, w4_buf, q_scr, sems, *, sk, w):
    S = _SLOTS
    scale = _DH ** -0.5
    offs4 = [int(o) for o in np.cumsum((0,) + _W4_SPLIT)]

    def start_head(h, slot):
        kc = _tiles(kt_hbm.at[h], k_buf.at[slot], 32, 512, sems.at[slot], c0=sk - w)
        vc = _tiles(vt_hbm.at[h], v_buf.at[slot], 32, 512, sems.at[S + slot], c0=sk - w)
        _start_alternating(_interleave(kc, vc))

    x_copy = pltpu.make_async_copy(x_hbm, x_buf, sems.at[2 * S])
    wq_sem, wo_sem, w3_sem = sems.at[2 * S + 1], sems.at[2 * S + 2], sems.at[2 * S + 3]

    def w4_part(c):
        rows = pl.ds(offs4[c], _W4_SPLIT[c])
        return w4_hbm.at[rows], w4_buf.at[rows], sems.at[2 * S + 4 + c]

    x_copy.start()
    _start_alternating(_interleave(_wo_tiles(wo_hbm, wo_buf, wo_sem),
                                   _slab_tiles(wq_hbm, wq_buf, 8, 256, wq_sem)))
    for h in range(S):
        start_head(h, h)

    x_copy.wait()
    x8 = jnp.broadcast_to(x_buf[0].astype(jnp.float32), (_M, _D))
    xn = _ln(x8).astype(jnp.bfloat16)
    _wait_filled(wq_buf, wq_sem)
    wq = wq_buf[...].reshape(_D, _H * _DH)
    q_all = jnp.dot(xn, wq, preferred_element_type=jnp.float32).astype(jnp.bfloat16)
    for h in range(_H):
        q_scr[h] = q_all[:, h * _DH:(h + 1) * _DH]
    _wait_filled(wo_buf, wo_sem)

    def head(h, acc):
        slot = h % S
        q = q_scr[h]
        _wait_filled(k_buf.at[slot], sems.at[slot])
        s = jnp.dot(q, k_buf[slot], preferred_element_type=jnp.float32) * scale
        m = jnp.max(s, axis=-1, keepdims=True)
        e = jnp.exp(s - m)
        l = jnp.sum(e, axis=-1, keepdims=True)
        _wait_filled(v_buf.at[slot], sems.at[S + slot])
        o = jax.lax.dot_general(e.astype(jnp.bfloat16), v_buf[slot], (((1,), (1,)), ((), ())),
                                preferred_element_type=jnp.float32)
        o = (o / l).astype(jnp.bfloat16)
        nblk = wo_buf.shape[1]
        wo = jnp.concatenate([wo_buf[(3 * h + b) // nblk, (3 * h + b) % nblk] for b in range(3)], axis=0)
        acc = acc + jnp.dot(o, wo, preferred_element_type=jnp.float32)

        @pl.when(h + S < _H)
        def _():
            start_head(h + S, slot)

        @pl.when(h + S == _H)
        def _():
            w4_tiles = [t for c in range(len(_W4_SPLIT)) for t in _tiles(*w4_part(c)[:2], 32, _D, w4_part(c)[2])]
            _start_alternating(_interleave(_slab_tiles(w3_hbm, w3_buf, 8, 256, w3_sem), w4_tiles))

        return acc

    attn = jax.lax.fori_loop(0, _H, head, jnp.zeros((_M, _D), jnp.float32))

    hres = x8 + attn
    x1 = _ln(hres)
    xn2 = _ln(x1).astype(jnp.bfloat16)
    _wait_filled(w3_buf, w3_sem)
    w3 = w3_buf[...].reshape(_D, _F)
    g = _gelu(jnp.dot(xn2, w3, preferred_element_type=jnp.float32)).astype(jnp.bfloat16)
    res = hres + x1
    for c in range(len(_W4_SPLIT)):
        _, dst, sem = w4_part(c)
        _wait_filled(dst, sem)
        res = res + jnp.dot(g[:, offs4[c]:offs4[c + 1]], dst[...], preferred_element_type=jnp.float32)
    out_ref[0] = res[0:1].astype(out_ref.dtype)


@jax.jit
def pallas_sequential_preLN__sliding_block_cached__mixer_s_mlp__decode_kernel(
    A_x: jax.Array,
    A_k_cache: jax.Array,
    A_v_cache: jax.Array,
    A_wq: jax.Array,
    A_wo: jax.Array,
    B_x: jax.Array,
    B_w1: jax.Array,
    B_w2: jax.Array,
    B_w3: jax.Array,
    B_w4: jax.Array,
):
    del B_x, B_w1, B_w2
    sk = A_k_cache.shape[2]
    w = min(4096, max(256, sk // 4))
    kt = jnp.swapaxes(A_k_cache, 2, 3).reshape(_H, _DH, sk)
    vt = jnp.swapaxes(A_v_cache, 2, 3).reshape(_H, _DH, sk)
    wq = A_wq.reshape(_WQ_SLABS, _D // _WQ_SLABS, _H * _DH)
    wo = A_wo.reshape(_WO_SLABS, _H * _DH // (64 * _WO_SLABS), 64, _D)
    w3 = B_w3.reshape(_W3_SLABS, _D // _W3_SLABS, _F)
    any_spec = pl.BlockSpec(memory_space=pl.ANY)
    return pl.pallas_call(
        functools.partial(_kernel, sk=sk, w=w),
        out_shape=jax.ShapeDtypeStruct((1, 1, _D), A_x.dtype),
        in_specs=[any_spec] * 7,
        out_specs=pl.BlockSpec(memory_space=pltpu.VMEM),
        scratch_shapes=[
            pltpu.VMEM((1, 1, _D), jnp.bfloat16),
            pltpu.VMEM(wq.shape, jnp.bfloat16),
            pltpu.VMEM((_SLOTS, _DH, w), jnp.bfloat16),
            pltpu.VMEM((_SLOTS, _DH, w), jnp.bfloat16),
            pltpu.VMEM(wo.shape, jnp.bfloat16),
            pltpu.VMEM(w3.shape, jnp.bfloat16),
            pltpu.VMEM((_F, _D), jnp.bfloat16),
            pltpu.VMEM((_H, _M, _DH), jnp.bfloat16),
            pltpu.SemaphoreType.DMA((2 * _SLOTS + 4 + len(_W4_SPLIT),)),
        ],
        compiler_params=pltpu.CompilerParams(vmem_limit_bytes=64 * 1024 * 1024,
                                             disable_semaphore_checks=True),
    )(A_x, kt, vt, wq, wo, w3, B_w4)
```

```python
import functools

import jax
import jax.numpy as jnp
import numpy as np
import jax.experimental.pallas as pl
import jax.experimental.pallas.tpu as pltpu

_H, _DH, _D, _F = 32, 192, 640, 1536
_M = 8
_EPS = 1e-5
_SLOTS = 2
_W4_SPLIT = (768, 384, 256, 128)
_WQ_SLABS, _WO_SLABS, _W3_SLABS = 10, 12, 10


def _ln(v):
    m = jnp.mean(v, axis=-1, keepdims=True)
    d = v - m
    var = jnp.mean(d * d, axis=-1, keepdims=True)
    return d * jax.lax.rsqrt(var + _EPS)


def _gelu(v):
    c = float(np.sqrt(2.0 / np.pi))
    return 0.5 * v * (1.0 + jnp.tanh(c * (v + 0.044715 * (v * v * v))))


def _tiles(src, dst, rb, cb, sem, c0=0):
    rows, cols = dst.shape
    return [pltpu.make_async_copy(src.at[pl.ds(r * rb, rb), pl.ds(c0 + c * cb, cb)],
                                  dst.at[pl.ds(r * rb, rb), pl.ds(c * cb, cb)], sem)
            for c in range(cols // cb) for r in range(rows // rb)]


def _slab_tiles(src, dst, rb, cb, sem):
    _, rows, cols = dst.shape
    return [pltpu.make_async_copy(src.at[:, pl.ds(r * rb, rb), pl.ds(c * cb, cb)],
                                  dst.at[:, pl.ds(r * rb, rb), pl.ds(c * cb, cb)], sem)
            for r in range(rows // rb) for c in range(cols // cb)]


def _wo_tiles(src, dst, sem):
    _, blocks, rows, cols = dst.shape
    return [pltpu.make_async_copy(src.at[:, b, pl.ds(r * 8, 8), pl.ds(c * 128, 128)],
                                  dst.at[:, b, pl.ds(r * 8, 8), pl.ds(c * 128, 128)], sem)
            for b in range(blocks) for r in range(rows // 8) for c in range(cols // 128)]


def _interleave(a, b):
    n = min(len(a), len(b))
    return [c for pair in zip(a[:n], b[:n]) for c in pair] + a[n:] + b[n:]


def _start_alternating(copies):
    for i, c in enumerate(copies):
        c.start(priority=i % 2)


def _wait_filled(buf, sem):
    pltpu.make_async_copy(buf, buf, sem).wait()


def _kernel(x_hbm, kt_hbm, vt_hbm, wq_hbm, wo_hbm, w3_hbm, w4_hbm, out_ref,
            x_buf, wq_buf, k_buf, v_buf, wo_buf, w3_buf, w4_buf, q_scr, sems, *, sk, w):
    S = _SLOTS
    scale = _DH ** -0.5
    offs4 = [int(o) for o in np.cumsum((0,) + _W4_SPLIT)]

    def start_head(h, slot):
        kc = _tiles(kt_hbm.at[h], k_buf.at[slot], 32, 512, sems.at[slot], c0=sk - w)
        vc = _tiles(vt_hbm.at[h], v_buf.at[slot], 32, 512, sems.at[S + slot], c0=sk - w)
        _start_alternating(_interleave(kc, vc))

    x_copy = pltpu.make_async_copy(x_hbm, x_buf, sems.at[2 * S])
    wq_sem, wo_sem, w3_sem = sems.at[2 * S + 1], sems.at[2 * S + 2], sems.at[2 * S + 3]

    w4_parts = []
    for c, n in enumerate(_W4_SPLIT):
        rows = pl.ds(offs4[c], n)
        w4_parts.append((w4_hbm.at[rows], w4_buf.at[rows], sems.at[2 * S + 4 + c]))

    x_copy.start()
    _start_alternating(_interleave(_wo_tiles(wo_hbm, wo_buf, wo_sem),
                                   _slab_tiles(wq_hbm, wq_buf, 8, 256, wq_sem)))
    for h in range(S):
        start_head(h, h)

    x_copy.wait()
    x8 = jnp.broadcast_to(x_buf[0].astype(jnp.float32), (_M, _D))
    xn = _ln(x8).astype(jnp.bfloat16)
    _wait_filled(wq_buf, wq_sem)
    wq = wq_buf[...].reshape(_D, _H * _DH)
    q_all = jnp.dot(xn, wq, preferred_element_type=jnp.float32).astype(jnp.bfloat16)
    for h in range(_H):
        q_scr[h] = q_all[:, h * _DH:(h + 1) * _DH]
    _wait_filled(wo_buf, wo_sem)

    def head(h, acc):
        slot = h % S
        q = q_scr[h]
        _wait_filled(k_buf.at[slot], sems.at[slot])
        s = jnp.dot(q, k_buf[slot], preferred_element_type=jnp.float32) * scale
        m = jnp.max(s, axis=-1, keepdims=True)
        e = jnp.exp(s - m)
        l = jnp.sum(e, axis=-1, keepdims=True)
        _wait_filled(v_buf.at[slot], sems.at[S + slot])
        o = jax.lax.dot_general(e.astype(jnp.bfloat16), v_buf[slot], (((1,), (1,)), ((), ())),
                                preferred_element_type=jnp.float32)
        o = (o / l).astype(jnp.bfloat16)
        nblk = wo_buf.shape[1]
        wo = jnp.concatenate([wo_buf[(3 * h + b) // nblk, (3 * h + b) % nblk] for b in range(3)], axis=0)
        acc = acc + jnp.dot(o, wo, preferred_element_type=jnp.float32)

        @pl.when(h + S < _H)
        def _():
            start_head(h + S, slot)

        @pl.when(h + S == _H)
        def _():
            w4_tiles = [t for src, dst, sem in w4_parts for t in _tiles(src, dst, 32, _D, sem)]
            _start_alternating(_interleave(_slab_tiles(w3_hbm, w3_buf, 8, 256, w3_sem), w4_tiles))

        return acc

    attn = jax.lax.fori_loop(0, _H, head, jnp.zeros((_M, _D), jnp.float32))

    hres = x8 + attn
    x1 = _ln(hres)
    xn2 = _ln(x1).astype(jnp.bfloat16)
    _wait_filled(w3_buf, w3_sem)
    w3 = w3_buf[...].reshape(_D, _F)
    g = _gelu(jnp.dot(xn2, w3, preferred_element_type=jnp.float32)).astype(jnp.bfloat16)
    res = hres + x1
    for c, (_, dst, sem) in enumerate(w4_parts):
        _wait_filled(dst, sem)
        res = res + jnp.dot(g[:, offs4[c]:offs4[c + 1]], dst[...], preferred_element_type=jnp.float32)
    out_ref[0] = res[0:1].astype(out_ref.dtype)


@jax.jit
def pallas_sequential_preLN__sliding_block_cached__mixer_s_mlp__decode_kernel(
    A_x: jax.Array,
    A_k_cache: jax.Array,
    A_v_cache: jax.Array,
    A_wq: jax.Array,
    A_wo: jax.Array,
    B_x: jax.Array,
    B_w1: jax.Array,
    B_w2: jax.Array,
    B_w3: jax.Array,
    B_w4: jax.Array,
):
    del B_x, B_w1, B_w2
    sk = A_k_cache.shape[2]
    w = min(4096, max(256, sk // 4))
    kt = jnp.swapaxes(A_k_cache, 2, 3).reshape(_H, _DH, sk)
    vt = jnp.swapaxes(A_v_cache, 2, 3).reshape(_H, _DH, sk)
    wq = A_wq.reshape(_WQ_SLABS, _D // _WQ_SLABS, _H * _DH)
    wo = A_wo.reshape(_WO_SLABS, _H * _DH // (64 * _WO_SLABS), 64, _D)
    w3 = B_w3.reshape(_W3_SLABS, _D // _W3_SLABS, _F)
    any_spec = pl.BlockSpec(memory_space=pl.ANY)
    return pl.pallas_call(
        functools.partial(_kernel, sk=sk, w=w),
        out_shape=jax.ShapeDtypeStruct((1, 1, _D), A_x.dtype),
        in_specs=[any_spec] * 7,
        out_specs=pl.BlockSpec(memory_space=pltpu.VMEM),
        scratch_shapes=[
            pltpu.VMEM((1, 1, _D), jnp.bfloat16),
            pltpu.VMEM(wq.shape, jnp.bfloat16),
            pltpu.VMEM((_SLOTS, _DH, w), jnp.bfloat16),
            pltpu.VMEM((_SLOTS, _DH, w), jnp.bfloat16),
            pltpu.VMEM(wo.shape, jnp.bfloat16),
            pltpu.VMEM(w3.shape, jnp.bfloat16),
            pltpu.VMEM((_F, _D), jnp.bfloat16),
            pltpu.VMEM((_H, _M, _DH), jnp.bfloat16),
            pltpu.SemaphoreType.DMA((2 * _SLOTS + 4 + len(_W4_SPLIT),)),
        ],
        compiler_params=pltpu.CompilerParams(vmem_limit_bytes=64 * 1024 * 1024,
                                             disable_semaphore_checks=True),
    )(A_x, kt, vt, wq, wo, w3, B_w4)
```

```python
import functools

import jax
import jax.numpy as jnp
import numpy as np
import jax.experimental.pallas as pl
import jax.experimental.pallas.tpu as pltpu

_H, _DH, _D, _F = 32, 192, 640, 1536
_M = 8
_EPS = 1e-5
_SLOTS = 2
_W4_SPLIT = (768, 384, 256, 128)
_WQ_SLABS, _WO_SLABS, _W3_SLABS = 10, 12, 10
_LEAD = 26


def _ln(v):
    m = jnp.mean(v, axis=-1, keepdims=True)
    d = v - m
    var = jnp.mean(d * d, axis=-1, keepdims=True)
    return d * jax.lax.rsqrt(var + _EPS)


def _gelu(v):
    c = float(np.sqrt(2.0 / np.pi))
    return 0.5 * v * (1.0 + jnp.tanh(c * (v + 0.044715 * (v * v * v))))


def _tiles(src, dst, rb, cb, sem, c0=0):
    rows, cols = dst.shape
    assert rows % rb == 0 and cols % cb == 0
    return [pltpu.make_async_copy(src.at[pl.ds(r * rb, rb), pl.ds(c0 + c * cb, cb)],
                                  dst.at[pl.ds(r * rb, rb), pl.ds(c * cb, cb)], sem)
            for c in range(cols // cb) for r in range(rows // rb)]


def _slab_tiles(src, dst, rb, cb, sem):
    _, rows, cols = dst.shape
    assert rows % rb == 0 and cols % cb == 0
    return [pltpu.make_async_copy(src.at[:, pl.ds(r * rb, rb), pl.ds(c * cb, cb)],
                                  dst.at[:, pl.ds(r * rb, rb), pl.ds(c * cb, cb)], sem)
            for r in range(rows // rb) for c in range(cols // cb)]


def _wo_tiles(src, dst, sem):
    _, blocks, rows, cols = dst.shape
    assert rows % 8 == 0 and cols % 128 == 0
    return [pltpu.make_async_copy(src.at[:, b, pl.ds(r * 8, 8), pl.ds(c * 128, 128)],
                                  dst.at[:, b, pl.ds(r * 8, 8), pl.ds(c * 128, 128)], sem)
            for b in range(blocks) for r in range(rows // 8) for c in range(cols // 128)]


def _interleave(a, b):
    n = min(len(a), len(b))
    return [c for pair in zip(a[:n], b[:n]) for c in pair] + a[n:] + b[n:]


def _start_alternating(copies):
    for i, c in enumerate(copies):
        c.start(priority=i % 2)


def _wait_filled(buf, sem):
    pltpu.make_async_copy(buf, buf, sem).wait()


def _kernel(x_hbm, kt_hbm, vt_hbm, wq_hbm, wo_hbm, w3_hbm, w4_hbm, out_ref,
            x_buf, wq_buf, k_buf, v_buf, wo_buf, w3_buf, w4_buf, q_scr, sems, *, sk, w):
    S = _SLOTS
    scale = _DH ** -0.5
    offs4 = [int(o) for o in np.cumsum((0,) + _W4_SPLIT)]

    def start_head(h, slot):
        kc = _tiles(kt_hbm.at[h], k_buf.at[slot], 32, 512, sems.at[slot], c0=sk - w)
        vc = _tiles(vt_hbm.at[h], v_buf.at[slot], 32, 512, sems.at[S + slot], c0=sk - w)
        _start_alternating(_interleave(kc, vc))

    x_copy = pltpu.make_async_copy(x_hbm, x_buf, sems.at[2 * S])
    wq_sem, wo_sem, w3_sem = sems.at[2 * S + 1], sems.at[2 * S + 2], sems.at[2 * S + 3]

    w4_parts = []
    for c, n in enumerate(_W4_SPLIT):
        rows = pl.ds(offs4[c], n)
        w4_parts.append((w4_hbm.at[rows], w4_buf.at[rows], sems.at[2 * S + 4 + c]))

    x_copy.start()
    wq_tiles = _slab_tiles(wq_hbm, wq_buf, 8, 256, wq_sem)
    for c in wq_tiles[:_LEAD]:
        c.start(priority=1)
    _start_alternating(_interleave(_wo_tiles(wo_hbm, wo_buf, wo_sem), wq_tiles[_LEAD:]))
    for h in range(S):
        start_head(h, h)

    x_copy.wait()
    x8 = jnp.broadcast_to(x_buf[0].astype(jnp.float32), (_M, _D))
    xn = _ln(x8).astype(jnp.bfloat16)
    _wait_filled(wq_buf, wq_sem)
    wq = wq_buf[...].reshape(_D, _H * _DH)
    q_all = jnp.dot(xn, wq, preferred_element_type=jnp.float32).astype(jnp.bfloat16)
    for h in range(_H):
        q_scr[h] = q_all[:, h * _DH:(h + 1) * _DH]
    _wait_filled(wo_buf, wo_sem)

    def head(h, acc):
        slot = h % S
        q = q_scr[h]
        _wait_filled(k_buf.at[slot], sems.at[slot])
        s = jnp.dot(q, k_buf[slot], preferred_element_type=jnp.float32) * scale
        m = jnp.max(s, axis=-1, keepdims=True)
        e = jnp.exp(s - m)
        l = jnp.sum(e, axis=-1, keepdims=True)
        _wait_filled(v_buf.at[slot], sems.at[S + slot])
        o = jax.lax.dot_general(e.astype(jnp.bfloat16), v_buf[slot], (((1,), (1,)), ((), ())),
                                preferred_element_type=jnp.float32)
        o = (o / l).astype(jnp.bfloat16)
        nblk = wo_buf.shape[1]
        wo = jnp.concatenate([wo_buf[(3 * h + b) // nblk, (3 * h + b) % nblk] for b in range(3)], axis=0)
        acc = acc + jnp.dot(o, wo, preferred_element_type=jnp.float32)

        @pl.when(h + S < _H)
        def _():
            start_head(h + S, slot)

        @pl.when(h + S == _H)
        def _():
            w4_tiles = [t for src, dst, sem in w4_parts for t in _tiles(src, dst, 32, _D, sem)]
            _start_alternating(_interleave(_slab_tiles(w3_hbm, w3_buf, 8, 256, w3_sem), w4_tiles))

        return acc

    attn = jax.lax.fori_loop(0, _H, head, jnp.zeros((_M, _D), jnp.float32))

    hres = x8 + attn
    x1 = _ln(hres)
    xn2 = _ln(x1).astype(jnp.bfloat16)
    _wait_filled(w3_buf, w3_sem)
    w3 = w3_buf[...].reshape(_D, _F)
    g = _gelu(jnp.dot(xn2, w3, preferred_element_type=jnp.float32)).astype(jnp.bfloat16)
    res = hres + x1
    for c, (_, dst, sem) in enumerate(w4_parts):
        _wait_filled(dst, sem)
        res = res + jnp.dot(g[:, offs4[c]:offs4[c + 1]], dst[...], preferred_element_type=jnp.float32)
    out_ref[0] = res[0:1].astype(out_ref.dtype)


@jax.jit
def pallas_sequential_preLN__sliding_block_cached__mixer_s_mlp__decode_kernel(
    A_x: jax.Array,
    A_k_cache: jax.Array,
    A_v_cache: jax.Array,
    A_wq: jax.Array,
    A_wo: jax.Array,
    B_x: jax.Array,
    B_w1: jax.Array,
    B_w2: jax.Array,
    B_w3: jax.Array,
    B_w4: jax.Array,
):
    del B_x, B_w1, B_w2
    sk = A_k_cache.shape[2]
    w = min(4096, max(256, sk // 4))
    kt = jnp.swapaxes(A_k_cache, 2, 3).reshape(_H, _DH, sk)
    vt = jnp.swapaxes(A_v_cache, 2, 3).reshape(_H, _DH, sk)
    wq = A_wq.reshape(_WQ_SLABS, _D // _WQ_SLABS, _H * _DH)
    wo = A_wo.reshape(_WO_SLABS, _H * _DH // (64 * _WO_SLABS), 64, _D)
    w3 = B_w3.reshape(_W3_SLABS, _D // _W3_SLABS, _F)
    any_spec = pl.BlockSpec(memory_space=pl.ANY)
    return pl.pallas_call(
        functools.partial(_kernel, sk=sk, w=w),
        out_shape=jax.ShapeDtypeStruct((1, 1, _D), A_x.dtype),
        in_specs=[any_spec] * 7,
        out_specs=pl.BlockSpec(memory_space=pltpu.VMEM),
        scratch_shapes=[
            pltpu.VMEM((1, 1, _D), jnp.bfloat16),
            pltpu.VMEM(wq.shape, jnp.bfloat16),
            pltpu.VMEM((_SLOTS, _DH, w), jnp.bfloat16),
            pltpu.VMEM((_SLOTS, _DH, w), jnp.bfloat16),
            pltpu.VMEM(wo.shape, jnp.bfloat16),
            pltpu.VMEM(w3.shape, jnp.bfloat16),
            pltpu.VMEM((_F, _D), jnp.bfloat16),
            pltpu.VMEM((_H, _M, _DH), jnp.bfloat16),
            pltpu.SemaphoreType.DMA((2 * _SLOTS + 4 + len(_W4_SPLIT),)),
        ],
        compiler_params=pltpu.CompilerParams(vmem_limit_bytes=64 * 1024 * 1024,
                                             disable_semaphore_checks=True),
    )(A_x, kt, vt, wq, wo, w3, B_w4)
```
